```python
import os as _os
_os.environ.setdefault("JAX_PLATFORMS", "cpu")
import jax
import jax.numpy as jnp

def _softmax(x, axis=-1):
    return jax.nn.softmax(x, axis=axis)
def _gelu(x):
    return jax.nn.gelu(x, approximate=True)
def _silu(x):
    return jax.nn.silu(x)
def _sigmoid(x):
    return jax.nn.sigmoid(x)
def _layernorm(x, axis=-1, eps=1e-5):
    m = jnp.mean(x, axis=axis, keepdims=True)
    v = jnp.var(x, axis=axis, keepdims=True)
    return (x - m) / jnp.sqrt(v + eps)
def _scatter_add(tgt, idx, src, axis=0):
    return tgt.at[idx].add(src)
def _segment_sum(src, seg, n):
    return jax.ops.segment_sum(src, seg, n)
class _Rng:
    def __init__(self, key):
        self._k = key
    def _next(self):
        self._k, sub = jax.random.split(self._k)
        return sub
    def normal(self, shape):
        return jax.random.normal(self._next(), shape, dtype=jnp.bfloat16)
    def randint(self, lo, hi, shape):
        return jax.random.randint(self._next(), shape, lo, hi, dtype=jnp.int32)
    def uniform(self, shape, lo=0.0, hi=1.0):
        return jax.random.uniform(self._next(), shape, jnp.bfloat16, lo, hi)
    def permutation(self, n):
        return jax.random.permutation(self._next(), n)


kernel_name = 'concat_heads__mha_block__spectral_gfnet__prompt'

def setup_inputs():
    _rng = _Rng(jax.random.key(int.from_bytes(__import__("os").urandom(4), "little")))
    _w = (lambda a: (lambda t: t.astype(jnp.bfloat16) if jnp.issubdtype(t.dtype, jnp.floating) else t)(jnp.asarray(a)))
    def _A_setup():
        B, S, D, H = 1, 2048, 512, 32
        return {
            "x": _w((lambda *s: _rng.normal(s) * 0.2)(B, S, D)),
            "wqkv": _w((lambda *s: _rng.normal(s) * 0.2)(D, 3 * D)),
            "wo": _w((lambda *s: _rng.normal(s) * 0.05)(D, D)),
        }
    _A_in = _A_setup()

    def _B_setup():
        B, S, D = 1, 2048, 512
        Df = D // 2 + 1
        return {
            "x": _w((lambda *s: _rng.normal(s) * 0.05)(B, S, D)),
            "w_r": _w((lambda *s: _rng.normal(s) * 0.05)(S, Df) * 0.02),
            "w_i": _w((lambda *s: _rng.normal(s) * 0.05)(S, Df) * 0.02),
        }
    _B_in = _B_setup()

    return {
        "A_x": _A_in["x"],
        "A_wqkv": _A_in["wqkv"],
        "A_wo": _A_in["wo"],
        "B_x": _B_in["x"],
        "B_w_r": _B_in["w_r"],
        "B_w_i": _B_in["w_i"],
    }

def reference(A_x, A_wqkv, A_wo, B_x, B_w_r, B_w_i):
    def _A_ref(x, wqkv, wo):
        B, S, D = x.shape
        H = 32
        Dh = D // H
        qkv = (lambda x, *d: x.transpose(*d))((x @ wqkv).reshape(B, S, 3, H, Dh), 2, 0, 3, 1, 4)
        q, k, v = qkv[0], qkv[1], qkv[2]
        scores = jnp.einsum("bhqd,bhkd->bhqk", q, k) * (Dh ** -0.5)
        p = _softmax(scores, axis=-1)
        o = jnp.einsum("bhqk,bhkd->bhqd", p, v)
        return (lambda x, *d: x.transpose(*d))(o, 0, 2, 1, 3).reshape(B, S, D) @ wo

    def _B_ref(x, w_r, w_i):
        B, S, D = x.shape
        X = (lambda x, axes=(-2,-1): jnp.fft.rfft2(x.astype(jnp.float32), axes=axes))(x, axes=(-2, -1))
        W = w_r + 1j * w_i
        X = X * W
        y = (lambda x, s, axes=(-2,-1): jnp.fft.irfft2(x, s=s, axes=axes).astype(jnp.bfloat16))(X, (S, D), axes=(-2, -1))
        return y

    a = _A_ref(A_x, A_wqkv, A_wo)
    b = _B_ref(B_x, B_w_r, B_w_i)
    return jnp.concatenate([a, b], axis=-1)
```

```python
import math

import jax
import jax.numpy as jnp
import numpy as np
from jax import lax
from jax.experimental import pallas as pl
from jax.experimental.pallas import tpu as pltpu

S, D, H, DH = 2048, 512, 32, 16
DF = D // 2 + 1
TQ = 512
TK = 256
HEADS_PER_ITER = 2
NA, NB = 32, 64

LOGIT_SCALE = DH ** -0.5 * math.log2(math.e)
QMAX = 3960.0
MAX_LOGIT = 64.0
MAX_SCALE_PRODUCT = 16.0
V_RANGE = 2.0 ** 40

F32, BF16 = jnp.float32, jnp.bfloat16


def _dft_constants():
    n = np.arange(128)[:, None]
    m = np.arange(64)[None, :]
    ang = lambda rows, k: 2 * np.pi * ((rows * k) % D) / D
    ee, eo = np.zeros((128, 128)), np.zeros((128, 128))
    ee[:, 0::2], ee[:, 1::2] = np.cos(ang(n, 4 * m)), -np.sin(ang(n, 4 * m))
    ee[:, 1] = (-1.0) ** n[:, 0]
    eo[:, 1::2], eo[:, 0::2] = np.cos(ang(n, 4 * m + 2)), np.roll(-np.sin(ang(n, 4 * m + 2)), 1, axis=1)
    n2, k_odd = np.arange(256)[:, None], 2 * np.arange(128)[None, :] + 1
    odd = np.concatenate([np.cos(ang(n2, k_odd)), -np.sin(ang(n2, k_odd))], axis=1)
    norm = 1.0 / (S * D)
    ee_w = np.full((128, 1), 2.0)
    ee_w[0] = ee_w[1] = 1.0
    d_even = np.stack([ee, eo, ee.T * ee_w * norm, eo.T * 2 * norm])
    d_odd = np.stack([odd, odd.T * 2 * norm])

    b = np.arange(NB)[None, None, :]
    k1 = np.arange(NA)[:, None, None] + NA * np.arange(NB)[None, :, None]
    th = 2 * np.pi * ((b * k1) % S) / S
    mr, mi = np.cos(th), -np.sin(th)
    fwd = np.concatenate([np.concatenate([mr, -mi], axis=2),
                          np.concatenate([mi, mr], axis=2)], axis=1)
    seq = np.stack([fwd, fwd.transpose(0, 2, 1)])

    a = np.arange(128)[:, None]
    c = np.arange(128)[None, :]
    live = a < NA
    th = 2 * np.pi * ((a * c) % NA) / NA
    ny_f = np.concatenate([np.cos(th) * live, -np.sin(th) * live], axis=1)
    ny_dft = np.stack([np.concatenate([ny_f, np.zeros_like(ny_f)], axis=0),
                       np.concatenate([ny_f.T, np.zeros_like(ny_f.T)], axis=1)])
    th = 2 * np.pi * (np.arange(NB)[:, None] * (c % NA)) / S
    ny_tw = np.stack([np.cos(th), -np.sin(th)]).astype(np.float32)
    to_bf16 = lambda m: m.astype(np.float32).astype(BF16)
    return (to_bf16(d_even), to_bf16(np.concatenate([d_odd, ny_dft])), to_bf16(seq), ny_tw)


_D_EVEN, _D_ODD, _SEQ, _NY_TW = _dft_constants()


def _cmul_const(z, k, n, sign):
    re, im = z
    k %= n
    if k == 0:
        return z
    c, s = math.cos(2 * math.pi * k / n), sign * math.sin(2 * math.pi * k / n)
    if (8 * k) % n == 0 and (4 * k) % n != 0:
        if c * s > 0:
            return (re - im) * c, (re + im) * c
        return (re + im) * c, (im - re) * c
    return re * c - im * s, re * s + im * c


def _fft(load, idx, sign):
    n = len(idx)
    if n == 1:
        return [load(idx[0])]
    if n == 2:
        (ar, ai), (br, bi) = load(idx[0]), load(idx[1])
        return [(ar + br, ai + bi), (ar - br, ai - bi)]
    ev = _fft(load, idx[0::2], sign)
    o1 = _fft(load, idx[1::4], sign)
    o3 = _fft(load, idx[3::4], sign)
    out = [None] * n
    for k in range(n // 4):
        ar, ai = _cmul_const(o1[k], k, n, sign)
        br, bi = _cmul_const(o3[k], 3 * k, n, sign)
        sr, si, dr, di = ar + br, ai + bi, ar - br, ai - bi
        (er, ei), (fr, fi) = ev[k], ev[k + n // 4]
        out[k] = (er + sr, ei + si)
        out[k + n // 2] = (er - sr, ei - si)
        plus, minus = (fr - di, fi + dr), (fr + di, fi - dr)
        out[k + n // 4], out[k + 3 * n // 4] = (plus, minus) if sign > 0 else (minus, plus)
    return out


def _dot(a, b, dims=((1,), (0,)), out=F32):
    return lax.dot_general(a, b, (dims, ((), ())), preferred_element_type=out)


def _digits(x):
    q = jnp.round(x).astype(jnp.int32)
    hi = (q + 128) >> 8
    lo = q - (hi << 8)
    return hi << 3, hi, lo, (lo + 8) >> 4


def _kernel(xa_hbm, wqkv_hbm, wo_hbm, xb_hbm, wr_hbm, wi_hbm, de_hbm, do_hbm, seq_hbm, tw_hbm,
            out_hbm,
            xa, wqkv, wo, xb, wr, wi, d_even, d_odd, seq, ny_tw,
            w_t, qkv_t, q_dig, k_dig, step, o_t, w_perm, z_buf, t_buf, out_a, out_b,
            in_sem, out_sem):
    copies = {}

    def fetch(name, src, dst):
        copies[name] = pltpu.make_async_copy(src, dst, in_sem.at[len(copies)])
        copies[name].start()

    def fetch_w(blk):
        cols = pl.ds(blk * 128, 128)
        fetch(("w", blk), wqkv_hbm.at[:, cols], wqkv.at[:, cols])

    def fetch_x(j):
        rows = pl.ds(j * TQ, TQ)
        fetch(("x", j), xa_hbm.at[rows], xa.at[rows])

    fetch_w(0)
    fetch_w(4)
    fetch_x(0)

    lane = lax.broadcasted_iota(jnp.int32, (8, 128), 1)

    def transpose_w(blk, row):
        copies["w", blk].wait()
        w_t[row:row + 128, :] = wqkv[:, blk * 128:(blk + 1) * 128].T

    def project(row, n_rows, j):
        cols = slice(j * TQ, (j + 1) * TQ)
        y = _dot(w_t[row:row + n_rows, :], xa[cols, :], ((1,), (1,)))
        qkv_t[row:row + n_rows, cols] = y
        return y

    def lane_tile_max(m):
        return jnp.maximum(jnp.maximum(m[:, 0:128], m[:, 128:256]),
                           jnp.maximum(m[:, 256:384], m[:, 384:512]))

    def make_digits(h, pair_q, pair_k):
        g, r = divmod(h, 8)
        mq = jnp.maximum(jnp.max(pair_q, axis=1, keepdims=True), 1e-30)
        mk = jnp.maximum(jnp.max(pair_k, axis=1, keepdims=True), 1e-30)
        mq, mk = jnp.broadcast_to(mq, (8, 128)), jnp.broadcast_to(mk, (8, 128))
        bound = jnp.sum(jnp.sqrt(mq) * jnp.sqrt(mk), axis=0, keepdims=True) * LOGIT_SCALE
        aq = jnp.sqrt(jnp.max(mq, axis=0, keepdims=True))
        ak = jnp.sqrt(jnp.max(mk, axis=0, keepdims=True))
        safe = (bound <= MAX_LOGIT) & (aq * ak * LOGIT_SCALE <= MAX_SCALE_PRODUCT)
        sq, sk = QMAX / aq, QMAX / ak
        step[h] = jnp.broadcast_to((256.0 * LOGIT_SCALE) / (sq * sk), (8, 128))
        for j in range(S // TQ):
            cols = slice(j * TQ, (j + 1) * TQ)
            row = 256 * g + DH * r
            top, hi, lo, mid = _digits(qkv_t[row:row + DH, cols] * jnp.tile(sq, (1, TQ // 128)))
            q_dig[h, :, cols] = jnp.concatenate(
                [top, top, lo, hi, mid, jnp.zeros_like(mid)], axis=0).astype(jnp.int8)
            row += 128
            top, hi, lo, mid = _digits(qkv_t[row:row + DH, cols] * jnp.tile(sk, (1, TQ // 128)))
            k_dig[h, cols, :] = jnp.concatenate(
                [top, top, top, top, hi, lo, mid, jnp.zeros_like(mid)],
                axis=0).astype(jnp.int16).T.astype(jnp.int8)
        return jnp.where(safe, 0.0, 1.0)

    unsafe = jnp.zeros((1, 128), F32)
    pair_max = {}
    for g in range(4):
        transpose_w(g, 256 * g)
        transpose_w(4 + g, 256 * g + 128)
        for j in range(4):
            if g == 0:
                if j < 3:
                    fetch_x(j + 1)
                if j == 2:
                    for blk in (1, 5, 2, 6, 3, 7, 8, 9, 10, 11):
                        fetch_w(blk)
                copies["x", j].wait()
            if g == 1 and j == 0:
                for name, src, dst in (("wr", wr_hbm, wr), ("wi", wi_hbm, wi), ("xb", xb_hbm, xb),
                                       ("wo", wo_hbm, wo), ("de", de_hbm, d_even), ("do", do_hbm, d_odd),
                                       ("seq", seq_hbm, seq), ("tw", tw_hbm, ny_tw)):
                    fetch(name, src, dst)
            y = project(256 * g, 256, j)
            y = y * y
            for i in range(16):
                m = lane_tile_max(y[16 * i:16 * i + 8] + y[16 * i + 8:16 * i + 16])
                pair_max[g, i] = m if j == 0 else jnp.maximum(pair_max[g, i], m)
            if g > 0:
                for r in (2 * j, 2 * j + 1):
                    unsafe += make_digits(8 * (g - 1) + r, pair_max[g - 1, r], pair_max[g - 1, 8 + r])
    for g in range(4):
        transpose_w(8 + g, 1024 + 128 * g)
    v_max = None
    for j in range(4):
        m = lane_tile_max(jnp.abs(project(1024, 512, j)))
        v_max = m if j == 0 else jnp.maximum(v_max, m)
        for r in (2 * j, 2 * j + 1):
            unsafe += make_digits(24 + r, pair_max[3, r], pair_max[3, 8 + r])
    v_max = jnp.max(v_max, axis=1, keepdims=True)
    v_ok = (v_max <= V_RANGE) & ((v_max >= 1.0 / V_RANGE) | (v_max == 0.0))
    n_unsafe = jnp.max(unsafe) + jnp.max(jnp.where(v_ok, 0.0, 1.0))

    @pl.when(n_unsafe == 0.0)
    def _():
        def body(it, carry):
            h0 = it * HEADS_PER_ITER
            steps = [(h0 + hh, j, t) for hh in range(HEADS_PER_ITER)
                     for j in range(S // TQ) for t in range(S // TK)]

            def logits(h, j, t):
                cols = slice(j * TQ, (j + 1) * TQ)
                starts = [t * TK + 128 * a + 32 * b for a in range(TK // 128) for b in (3, 2, 1, 0)]
                keys = jnp.concatenate([k_dig[h, s0:s0 + 32, :] for s0 in starts], axis=0)
                top = q_dig[h, 0:32, cols]
                return _dot(keys, jnp.concatenate([top, top, q_dig[h, 32:96, cols]], axis=0),
                            out=jnp.int32)

            y_next = logits(*steps[0])
            for n, (h, j, t) in enumerate(steps):
                y = y_next
                if n + 1 < len(steps):
                    y_next = logits(*steps[n + 1])
                c = jnp.tile(step[h], (1, TQ // 128))
                p = jnp.exp2(y.astype(F32).reshape(TK // 8, 8, TQ) * c)
                part = jnp.sum(p, axis=0)
                p = p.reshape(TK, TQ)
                p = jnp.concatenate([p[128 * a + 32 * b:128 * a + 32 * b + 32]
                                     for a in range(TK // 128) for b in (3, 2, 1, 0)], axis=0)
                rows = pl.ds(pl.multiple_of(1024 + h * DH, DH), DH)
                pv = _dot(qkv_t[rows, t * TK:(t + 1) * TK], p)
                den = part if t == 0 else den + part
                acc = pv if t == 0 else pv + acc
                if t == S // TK - 1:
                    o_t[pl.ds(pl.multiple_of(h * DH, DH), DH), j * TQ:(j + 1) * TQ] = (
                        acc * (1.0 / jnp.sum(den, axis=0, keepdims=True)))
            return carry

        lax.fori_loop(0, H // HEADS_PER_ITER, body, 0)

    @pl.when(n_unsafe != 0.0)
    def _():
        def body(it, carry):
            h, j = it // (S // TQ), it % (S // TQ)
            cols = pl.ds(pl.multiple_of(j * TQ, TQ), TQ)
            row = 256 * (h // 8) + DH * (h % 8)
            q = qkv_t[pl.ds(pl.multiple_of(row, DH), DH), cols]
            k = qkv_t[pl.ds(pl.multiple_of(row + 128, DH), DH), :]
            v = qkv_t[pl.ds(pl.multiple_of(1024 + h * DH, DH), DH), :]
            s = _dot(k.astype(BF16), q.astype(BF16), ((0,), (0,)))
            p = jnp.exp2((s - jnp.max(s, axis=0, keepdims=True)) * LOGIT_SCALE)
            o_t[pl.ds(pl.multiple_of(h * DH, DH), DH), cols] = (
                _dot(v, p) / jnp.sum(p, axis=0, keepdims=True))
            return carry

        lax.fori_loop(0, H * (S // TQ), body, 0)

    for name in ("wr", "wi", "xb", "wo", "de", "do", "seq", "tw"):
        copies[name].wait()
    out_copies = []

    def emit(buf, rows, col0):
        cp = pltpu.make_async_copy(buf.at[rows], out_hbm.at[rows, pl.ds(col0, D)],
                                   out_sem.at[len(out_copies)])
        cp.start()
        out_copies.append(cp)

    def project_out(i):
        rows = slice(128 * i, 128 * (i + 1))
        out_a[rows, :] = _dot(o_t[:, rows].T, wo[...]).astype(BF16)
        if i % 4 == 3:
            emit(out_a, pl.ds(512 * (i // 4), 512), 0)

    def wide(n_rows):
        return lax.broadcasted_iota(jnp.int32, (n_rows, 128), 1)

    CH = 256
    ny = jnp.zeros((NB, 128), F32)
    ny_w = [[], []]
    for i in range(S // CH):
        rows = slice(CH * i, CH * (i + 1))
        x0, x1, x2, x3 = (xb[rows, 128 * t:128 * (t + 1)].astype(F32) for t in range(4))
        s0, s1 = x0 + x2, x1 + x3
        ee = _dot(s0 + s1, d_even[0])
        eo = _dot(s0 - s1, d_even[1])
        od = _dot(jnp.concatenate([x0 - x2, x1 - x3], axis=1), d_odd[0])
        low = (wide(CH) & 1) == 0
        im = pltpu.roll(jnp.where(low, eo, ee), 127, 1)
        z_buf[0, rows, :] = jnp.where(low, ee, eo)
        z_buf[1, rows, :] = jnp.where(wide(CH) == 0, 0.0, im)
        z_buf[2, rows, :] = od[:, :128]
        z_buf[3, rows, :] = od[:, 128:]
        for a in range(CH // NB * i, CH // NB * (i + 1)):
            blk = im[NB * a - CH * i:NB * (a + 1) - CH * i]
            ny = jnp.where(wide(NB) == a, pltpu.roll(blk, a, 1) if a else blk, ny)
        for part, w in enumerate((wr, wi)):
            words = pltpu.bitcast(w[0:256, rows], jnp.int32).T
            for e in range(CH // NA):
                for c8 in range(NA // 8):
                    dst = 8 * (CH // NA * i + e)
                    w_perm[part, c8, dst:dst + 8, :] = words[NA * e + 8 * c8:NA * e + 8 * c8 + 8]
            last = jnp.broadcast_to(w[256:257, rows].astype(F32), (8, CH))
            sub = lax.broadcasted_iota(jnp.int32, (8, 128), 0)
            ny_w[part].append(jnp.where((lane >> 5) == (sub & 3),
                                        jnp.where(sub < 4, last[:, :128], last[:, 128:]), 0.0))

    for i in range(16):
        tile, r = divmod(i, NB // 8)
        res = _fft(lambda a: (z_buf[2 * tile, NB * a + 8 * r:NB * a + 8 * r + 8, :],
                              z_buf[2 * tile + 1, NB * a + 8 * r:NB * a + 8 * r + 8, :]),
                   list(range(NA)), -1)
        for c, (re, im) in enumerate(res):
            t_buf[c, 8 * r:8 * r + 8, 128 * tile:128 * (tile + 1)] = re
            t_buf[c, NB + 8 * r:NB + 8 * r + 8, 128 * tile:128 * (tile + 1)] = im
        if i % 2 == 1:
            project_out(i // 2)

    def cmul(ar, ai, br, bi):
        return ar * br - ai * bi, ar * bi + ai * br

    t = _dot(ny, d_odd[2, 0:128, :])
    x = _dot(seq[0, 0], jnp.concatenate(cmul(t[:, :128], t[:, 128:], ny_tw[0], ny_tw[1]), axis=0))
    y = cmul(x[:NB], x[NB:], jnp.concatenate(ny_w[0], axis=0), jnp.concatenate(ny_w[1], axis=0))
    t = _dot(seq[1, 0], jnp.concatenate(y, axis=0))
    ny = _dot(jnp.concatenate(cmul(t[:NB], t[NB:], ny_tw[0], -ny_tw[1]), axis=1), d_odd[3, :, 0:128])

    def spectrum(c2):
        return [_dot(seq[0, c], t_buf[c]) for c in (2 * c2, 2 * c2 + 1)]

    x_next = spectrum(0)
    for c2 in range(NA // 2):
        xs = x_next
        if c2 + 1 < NA // 2:
            x_next = spectrum(c2 + 1)
        for odd, x in enumerate(xs):
            c = 2 * c2 + odd
            words = [w_perm[part, c // 8, pl.ds(c % 8, NB, stride=8), :] for part in range(2)]
            y = cmul(x[:NB], x[NB:], *(jnp.concatenate(
                [pltpu.bitcast(w << 16, F32), pltpu.bitcast(w & -65536, F32)], axis=1) for w in words))
            t_buf[2 * c2 + odd] = _dot(seq[1, 2 * c2 + odd], jnp.concatenate(y, axis=0))

    for i in range(16):
        tile, r = divmod(i, NB // 8)
        res = _fft(lambda c: (t_buf[c, 8 * r:8 * r + 8, 128 * tile:128 * (tile + 1)],
                              t_buf[c, NB + 8 * r:NB + 8 * r + 8, 128 * tile:128 * (tile + 1)]),
                   list(range(NA)), 1)
        for a, (re, im) in enumerate(res):
            z_buf[2 * tile, NB * a + 8 * r:NB * a + 8 * r + 8, :] = re
            z_buf[2 * tile + 1, NB * a + 8 * r:NB * a + 8 * r + 8, :] = im
        if i % 2 == 1:
            project_out(8 + i // 2)

    for i in range(S // CH):
        rows = slice(CH * i, CH * (i + 1))
        nyq = jnp.concatenate([pltpu.roll(ny, 128 - a, 1) if a else ny
                               for a in range(CH // NB * i, CH // NB * (i + 1))], axis=0)
        re = z_buf[0, rows, :]
        im = pltpu.roll(jnp.where(wide(CH) == 0, nyq, z_buf[1, rows, :]), 1, 1)
        low = (wide(CH) & 1) == 0
        ee = _dot(jnp.where(low, re, im), d_even[2])
        eo = _dot(jnp.where(low, im, re), d_even[3])
        od = _dot(jnp.concatenate([z_buf[2, rows, :], z_buf[3, rows, :]], axis=1), d_odd[1])
        s0, s1, d0, d1 = ee + eo, ee - eo, od[:, :128], od[:, 128:]
        out_b[rows, :] = jnp.concatenate([s0 + d0, s1 + d1, s0 - d0, s1 - d1], axis=1).astype(BF16)
        emit(out_b, pl.ds(CH * i, CH), D)

    for cp in out_copies:
        cp.wait()


@jax.jit
def pallas_concat_heads__mha_block__spectral_gfnet__prompt_kernel(
    A_x: jax.Array,
    A_wqkv: jax.Array,
    A_wo: jax.Array,
    B_x: jax.Array,
    B_w_r: jax.Array,
    B_w_i: jax.Array,
):
    vmem = pltpu.VMEM
    out = pl.pallas_call(
        _kernel,
        out_shape=jax.ShapeDtypeStruct((S, 2 * D), BF16),
        in_specs=[pl.BlockSpec(memory_space=pltpu.HBM)] * 10,
        out_specs=pl.BlockSpec(memory_space=pltpu.HBM),
        scratch_shapes=[
            vmem((S, D), BF16), vmem((D, 3 * D), BF16), vmem((D, D), BF16), vmem((S, D), BF16),
            vmem((DF, S), BF16), vmem((DF, S), BF16),
            vmem(_D_EVEN.shape, BF16), vmem(_D_ODD.shape, BF16), vmem(_SEQ.shape, BF16),
            vmem(_NY_TW.shape, F32),
            vmem((3 * D, D), BF16), vmem((3 * D, S), F32),
            vmem((H, 96, S), jnp.int8), vmem((H, S, 128), jnp.int8), vmem((H, 8, 128), F32),
            vmem((D, S), F32), vmem((2, NA // 8, 8 * NB, 128), jnp.int32), vmem((4, S, 128), F32),
            vmem((NA, 2 * NB, 256), F32), vmem((S, D), BF16), vmem((S, D), BF16),
            pltpu.SemaphoreType.DMA((24,)), pltpu.SemaphoreType.DMA((12,)),
        ],
        compiler_params=pltpu.CompilerParams(vmem_limit_bytes=100 * 2 ** 20),
        name="mha_gfnet",
    )(A_x.reshape(S, D), A_wqkv, A_wo, B_x.reshape(S, D), B_w_r.T, B_w_i.T,
      _D_EVEN, _D_ODD, _SEQ, _NY_TW)
    return out.reshape(1, S, 2 * D)
```

```python
import math

import jax
import jax.numpy as jnp
import numpy as np
from jax import lax
from jax.experimental import pallas as pl
from jax.experimental.pallas import tpu as pltpu

F32, BF16, I32 = jnp.float32, jnp.bfloat16, jnp.int32

S, D, H, DH = 2048, 512, 32, 16
TQ = 512
TK = 256
HEADS_PER_ITER = 4
NA, NB = 32, 64
HA = NA // 2

LOGIT_SCALE = DH ** -0.5 * math.log2(math.e)
QMAX = 3940.0
TINY = 1e-30
MAX_UNIT = 2.0 ** -12
MIN_DENOM, MAX_DENOM, MAX_FINITE = 2.0 ** -20, 2.0 ** 100, 3e38

PROJECTION_PLAN = ("kk", "dkkkk", "qdvvvq", "qq" + "dvvkqq" + "kdvvkqq" * 3 + "kdvvkqqqq" + "kdvvv")
EARLY_OUT = 6
NYQUIST_AT = (0, 2, 14, 16)
SKIP_OUT = (0, 2, 4, 6)


def _dft_constants():
    def row_pairs(m):
        bits = m.astype(np.float32).astype(BF16).view(np.uint16).astype(np.uint32)
        return (bits[..., 0::2, :] | (bits[..., 1::2, :] << 16)).view(np.int32)

    n, m, l = np.arange(128)[:, None], np.arange(64)[None, :], np.arange(128)[None, :]
    angle = lambda k: 2 * np.pi * ((n * k) % D) / D
    ee, eo = np.zeros((128, 128)), np.zeros((128, 128))
    ee[:, 0::2], ee[:, 1::2] = np.cos(angle(4 * m)), -np.sin(angle(4 * m))
    ee[:, 1] = (-1.0) ** n[:, 0]
    eo[:, 1::2] = np.cos(angle(4 * m + 2))
    eo[:, 0::2] = np.roll(-np.sin(angle(4 * m + 2)), 1, axis=1)
    ga, gb = np.cos(angle(2 * l + 1)), -np.sin(angle(2 * l + 1)) * (-1.0) ** l
    twice = 2.0 / (S * D)
    ee_weight = np.where(n < 2, twice / 2, twice)
    forward = [ee, eo, ga, gb - ga, -(ga + gb)]
    inverse = [ee.T * ee_weight, eo.T * twice, gb.T * twice, (ga - gb).T * twice, -(ga + gb).T * twice]

    freq = np.arange(NA)[:, None, None] + NA * np.arange(NB)[None, :, None]
    th = 2 * np.pi * ((freq * np.arange(NB)[None, None, :]) % S) / S
    re, im = np.cos(th), -np.sin(th)
    seq = np.concatenate([np.concatenate([re, -im], axis=2), np.concatenate([im, re], axis=2)], axis=1)

    live = (n < NA) & (n // HA == l % 2)
    th = 2 * np.pi * (((n % HA) * l) % NA) / NA
    ny_re, ny_im = np.cos(th) * live, -np.sin(th) * live
    th = 2 * np.pi * (np.arange(NB)[:, None] * (l % NA)) / S
    return (row_pairs(np.stack(forward + inverse + [ny_re, ny_im, ny_re.T, ny_im.T])),
            row_pairs(np.stack([seq, seq.transpose(0, 2, 1)])),
            np.stack([np.cos(th), -np.sin(th)]).astype(np.float32))


_FEAT, _SEQ, _NY_TW = _dft_constants()


def _rotate(z, k, n, sign):
    re, im = z
    if k == 0:
        return z
    if 4 * k == n:
        return (-im, re) if sign > 0 else (im, -re)
    c, s = math.cos(2 * math.pi * k / n), sign * math.sin(2 * math.pi * k / n)
    if (8 * k) % n == 0 and (4 * k) % n != 0:
        return ((re - im) * c, (re + im) * c) if c * s > 0 else ((re + im) * c, (im - re) * c)
    return re * c - im * s, re * s + im * c


def _fft(load, idx, sign):
    n = len(idx)
    if n == 1:
        return [load(idx[0])]
    if n == 2:
        (ar, ai), (br, bi) = load(idx[0]), load(idx[1])
        return [(ar + br, ai + bi), (ar - br, ai - bi)]
    even, odd1, odd3 = (_fft(load, part, sign) for part in (idx[0::2], idx[1::4], idx[3::4]))
    out = [None] * n
    for k in range(n // 4):
        ar, ai = _rotate(odd1[k], k, n, sign)
        br, bi = _rotate(odd3[k], 3 * k, n, sign)
        sr, si, dr, di = ar + br, ai + bi, ar - br, ai - bi
        (er, ei), (fr, fi) = even[k], even[k + n // 4]
        out[k], out[k + n // 2] = (er + sr, ei + si), (er - sr, ei - si)
        plus, minus = (fr - di, fi + dr), (fr + di, fi - dr)
        out[k + n // 4], out[k + 3 * n // 4] = (plus, minus) if sign > 0 else (minus, plus)
    return out


def _fft_load_order(idx):
    if len(idx) <= 2:
        return idx
    return _fft_load_order(idx[0::2]) + _fft_load_order(idx[1::4]) + _fft_load_order(idx[3::4])


def _cmul(ar, ai, br, bi):
    return ar * br - ai * bi, ar * bi + ai * br


def _dot(a, b, contract=((1,), (0,)), out=F32):
    return lax.dot_general(a, b, (contract, ((), ())), preferred_element_type=out)


def _span(i, size):
    return pl.ds(i * size if isinstance(i, int) else pl.multiple_of(i * size, size), size)


def _group(v, i):
    return v[8 * i:8 * i + 8]


def _bf16(words):
    return pltpu.bitcast(words, BF16)


def _abs_max(t):
    return jnp.maximum(jnp.abs(t[:8]), jnp.abs(t[8:]))


def _digits(x):
    q = jnp.round(x).astype(I32)
    u = q + 128
    hi = u >> 8
    return hi << 3, hi, q, ((u & 255) - 120) >> 4


def _flip_groups(p):
    return jnp.concatenate([_group(p, 16 * a + g) for a in range(p.shape[0] // 128)
                            for g in range(15, -1, -1)], axis=0)


def _kernel(xa_hbm, wqkv_hbm, wo_hbm, xb_hbm, wr_hbm, wi_hbm, feat_hbm, seq_hbm, tw_hbm, out_hbm,
            xa, wqkv, wo, xb, wr, wi, feat, seq, ny_tw,
            w_t, k_t, v_t, q_dig, k_dig, q_max, k_unit, o_t,
            w_cls, t_buf, ny_buf, out_a, out_b, fence_buf, sem):
    def copy(src, dst, slot):
        return pltpu.make_async_copy(src, dst, sem.at[slot])

    def x_rows(lo, hi):
        return xa_hbm.at[pl.ds(lo, hi - lo)], xa.at[pl.ds(lo, hi - lo)]

    def w_part(part):
        return wqkv_hbm.at[:, _span(part, D)], wqkv.at[part]

    arrivals = [[copy(src, dst, slot) for src, dst in pairs] for slot, pairs in enumerate((
        [x_rows(0, 256), w_part(1)],
        [x_rows(256, 768)],
        [w_part(0), w_part(2)],
        [x_rows(768, S)],
        [(wr_hbm, wr), (wi_hbm, wi), (xb_hbm, xb), (wo_hbm, wo), (feat_hbm, feat), (seq_hbm, seq),
         (tw_hbm, ny_tw)]))]
    for batch in arrivals:
        for cp in batch:
            cp.start()

    def arrive(slot):
        for cp in arrivals[slot]:
            cp.wait()

    def fence():
        def body(i, carry):
            fence_buf[i] = i
            return carry

        lax.fori_loop(0, 2, body, 0)

    def transpose_weights(part):
        for blk in range(D // 128):
            w_t[part, _span(blk, 64), :] = pltpu.bitcast(wqkv[part, :, _span(blk, 128)].T, I32)

    def project(part, x):
        return _dot(_bf16(w_t[part]), x, ((1,), (1,)))

    def queries(n):
        cols = _span(n, 128)
        y = project(0, xa[cols, :])
        for h in range(H):
            q = y[DH * h:DH * (h + 1)]
            m = jnp.maximum(jnp.max(_abs_max(q), axis=0, keepdims=True), TINY)
            q_max[h, :, cols] = jnp.broadcast_to(m, (8, 128))
            top, hi, lo, mid = _digits(q * (pltpu.reciprocal(m, approx=True) * QMAX))
            q_dig[h, :, cols] = jnp.concatenate(
                [top, top, lo, hi, mid, jnp.zeros_like(mid)], axis=0).astype(jnp.int8)

    def keys(n):
        k_t[:, _span(n, 128)] = project(1, jnp.concatenate(
            [xa[_span(16 * n + g, 8), :].astype(F32) for g in range(15, -1, -1)], axis=0))

    def values(n):
        v_t[:, _span(n, 128)] = pltpu.bitcast(project(2, xa[_span(n, 128), :]).astype(BF16), I32)

    def key_digits(t):
        cols = _span(t, TK)
        scales = []
        for g in range(H // 8):
            m = []
            for h in range(8 * g, 8 * g + 8):
                a = _abs_max(k_t[_span(h, DH), cols])
                m.append(jnp.max(jnp.maximum(a[:, :128], a[:, 128:]), axis=0, keepdims=True))
            m = jnp.max(jnp.concatenate(m, axis=0), axis=1, keepdims=True)
            m = jnp.maximum(jnp.broadcast_to(m, (8, 128)), TINY)
            k_unit[t, _span(g, 8), :] = m * (256.0 * LOGIT_SCALE / QMAX ** 2)
            scales.append(pltpu.reciprocal(m, approx=True) * QMAX)
        for h in range(H):
            scale = jnp.tile(scales[h // 8][h % 8:h % 8 + 1], (1, TK // 128))
            top, hi, lo, mid = _digits(k_t[_span(h, DH), cols] * scale)
            k_dig[h, cols, :] = jnp.concatenate(
                [top, top, top, top, hi, lo, mid, jnp.zeros_like(mid)],
                axis=0).astype(jnp.int16).T.astype(jnp.int8)

    tasks = dict(q=queries, k=keys, v=values, d=key_digits)
    done = dict(q=0, k=0, v=0, d=0)
    for slot, new_weights in enumerate(((1,), (), (0, 2), ())):
        arrive(slot)
        for part in new_weights:
            transpose_weights(part)
        if slot == 3:
            fence()
        for name in PROJECTION_PLAN[slot]:
            assert name != "d" or 128 * done["k"] >= TK * (done["d"] + 1)
            tasks[name](done[name])
            done[name] += 1
    assert done == dict(q=S // 128, k=S // 128, v=S // 128, d=S // TK)
    arrive(4)

    def logits(h, j, t):
        top = q_dig[h, 0:32, _span(j, TQ)]
        digits = jnp.concatenate([top, top, q_dig[h, 32:96, _span(j, TQ)]], axis=0)
        return _dot(k_dig[h, _span(t, TK), :], digits, out=I32)

    def attend(it, failed):
        n_freq = S * HEADS_PER_ITER // H
        for part, w in enumerate((wr, wi)):
            words = pltpu.bitcast(w[0:D // 2, _span(it, n_freq)], I32).T
            for e in range(n_freq // NA):
                for c8 in range(NA // 8):
                    w_cls[part, c8, _span(it * (n_freq // NA) + e, 8), :] = _group(words, NA // 8 * e + c8)

        steps = [(it * HEADS_PER_ITER + i, j, t) for i in range(HEADS_PER_ITER)
                 for j in range(S // TQ) for t in range(S // TK)]
        y_next = logits(*steps[0])
        for n, (h, j, t) in enumerate(steps):
            y = y_next
            if n + 1 < len(steps):
                y_next = logits(*steps[n + 1])
            unit_k = jnp.broadcast_to(k_unit[t, pl.ds(h, 1), :], (8, 128))
            unit = q_max[h, :, _span(j, TQ)] * jnp.tile(unit_k, (1, TQ // 128))
            p = jnp.exp2(y.astype(F32).reshape(TK // 8, 8, TQ) * unit)
            den = jnp.sum(p, axis=0) if t == 0 else den + jnp.sum(p, axis=0)
            pv = _dot(_bf16(v_t[_span(h, DH // 2), _span(t, TK)]), _flip_groups(p.reshape(TK, TQ)))
            acc = pv if t == 0 else pv + acc
            coarsest = unit_k if t == 0 else jnp.maximum(coarsest, unit_k)
            if t == S // TK - 1:
                den = jnp.sum(den, axis=0, keepdims=True)
                o_t[_span(h, DH), _span(j, TQ)] = acc * (1.0 / den)
                ok = ((den >= MIN_DENOM) & (den <= MAX_DENOM) & (_abs_max(acc) <= MAX_FINITE)
                      & (q_max[h, :, _span(j, TQ)] * jnp.tile(coarsest, (1, TQ // 128)) <= MAX_UNIT))
                bad = jnp.where(ok, 0.0, 1.0)
                failed = failed + ((bad[:, 0:128] + bad[:, 128:256]) + (bad[:, 256:384] + bad[:, 384:512]))
        return failed

    failed = lax.fori_loop(0, H // HEADS_PER_ITER, attend, jnp.zeros((8, 128), F32))

    @pl.when(jnp.max(failed) > 0.0)
    def _():
        def attend_with_row_max(i, carry):
            h, cols = i // (S // TQ), _span(i % (S // TQ), TQ)
            q = _dot(_bf16(w_t[0, _span(h, DH // 2), :]), xa[cols, :], ((1,), (1,))).astype(BF16)

            def step(t, state):
                m_old, den, acc = state
                s = _dot(k_t[_span(h, DH), _span(t, TK)].astype(BF16), q, ((0,), (0,)))
                m = jnp.maximum(m_old, jnp.max(s, axis=0, keepdims=True))
                p = jnp.exp2((s - m) * LOGIT_SCALE)
                keep = jnp.exp2((m_old - m) * LOGIT_SCALE)
                pv = _dot(_bf16(v_t[_span(h, DH // 2), _span(t, TK)]), _flip_groups(p))
                return m, den * keep + jnp.sum(p, axis=0, keepdims=True), acc * keep + pv

            _, den, acc = lax.fori_loop(0, S // TK, step, (
                jnp.full((1, TQ), -jnp.inf, F32), jnp.zeros((1, TQ), F32), jnp.zeros((DH, TQ), F32)))
            o_t[_span(h, DH), cols] = acc / den
            return carry

        lax.fori_loop(0, H * (S // TQ), attend_with_row_max, 0)

    def out_a_copy(i):
        return copy(out_a.at[_span(i, 2)], out_hbm.at[_span(i, 2), :, pl.ds(0, D)], 0)

    def out_b_copy(r):
        return copy(out_b.at[r], out_hbm.at[:, _span(r, 8), pl.ds(D, D)], 0)

    def out_projection(first, last):
        for i in range(first, last):
            o = o_t[:, _span(i, 128)].astype(BF16).T
            for half in range(2):
                y = _dot(o, wo[:, _span(half, D // 2)]).astype(BF16)
                out_a[_span(i, 2), :, _span(half, D // 2)] = y.reshape(2, NB, D // 2)
                if half:
                    out_a_copy(i).start()
                yield

    lane = lax.broadcasted_iota(I32, (8, 128), 1)
    lanes = lax.broadcasted_iota(I32, (8 * HA, 128), 1)
    even_lane = (lanes & 1) == 0
    lane_sign = jnp.where(even_lane, 1.0, -1.0)

    def class_rows(m, parity, part, r, tile):
        return 2 * m + parity, _span(NB // 8 * part + r, 8), _span(tile, 128)

    order = _fft_load_order(list(range(HA)))
    pieces = out_projection(0, EARLY_OUT)
    for r in range(NB // 8):
        def tokens(first):
            return jnp.concatenate(
                [xb[_span(NB // 8 * (first + a) + r, 8), :].astype(F32) for a in order], axis=0)

        nyquist = jnp.zeros((8, 128), F32)
        for parity in range(2):
            x = tokens(0) - tokens(HA) if parity else tokens(0) + tokens(HA)
            x0, x1, x2, x3 = (x[:, 128 * i:128 * (i + 1)] for i in range(4))
            s0, s1, za, zb = x0 + x2, x1 + x3, x0 - x2, x3 - x1
            shared = _dot(za + zb, _bf16(feat[2]))
            odd_im = (_dot(za, _bf16(feat[3])) + shared) * lane_sign
            odd_re = _dot(zb, _bf16(feat[4])) + shared
            ee = _dot(s0 + s1, _bf16(feat[0]))
            eo = _dot(s0 - s1, _bf16(feat[1]))
            even_im = pltpu.roll(jnp.where(even_lane, eo, ee), 127, 1)
            for i, a in enumerate(order):
                slot, rows = HA * parity + a, _group(even_im, i)
                nyquist = jnp.where(lane == slot, pltpu.roll(rows, slot, 1) if slot else rows, nyquist)
            even = (jnp.where(even_lane, ee, eo), jnp.where(lanes == 0, 0.0, even_im))
            for tile, z in enumerate((even, (odd_re, odd_im))):
                spectrum = _fft(lambda a: _rotate([_group(v, order.index(a)) for v in z], a * parity, NA, -1),
                                list(range(HA)), -1)
                for m in range(HA):
                    for part in range(2):
                        t_buf[class_rows(m, parity, part, r, tile)] = spectrum[m][part]
            if 2 * r + parity not in SKIP_OUT:
                next(pieces)
        ny_buf[_span(r, 8), :] = nyquist
    assert next(pieces, "done") == "done"
    fence()

    def nyquist_filter(w):
        row = lax.broadcasted_iota(I32, (8, 128), 0)
        out = []
        for i in range(NB // 8):
            v = jnp.broadcast_to(w[D // 2:D // 2 + 1, _span(i, 256)].astype(F32), (8, 256))
            out.append(jnp.where((lane >> 5) == (row & 3), jnp.where(row < 4, v[:, :128], v[:, 128:]), 0.0))
        return jnp.concatenate(out, axis=0)

    def nyquist_column():
        v = _dot(ny_buf[...], jnp.concatenate([_bf16(feat[10]), _bf16(feat[11])], axis=1))
        yield
        v = _dot(_bf16(seq[0, 0]), jnp.concatenate(_cmul(v[:, :128], v[:, 128:], ny_tw[0], ny_tw[1]), axis=0))
        yield
        v = _dot(_bf16(seq[1, 0]), jnp.concatenate(
            _cmul(v[:NB], v[NB:], nyquist_filter(wr), nyquist_filter(wi)), axis=0))
        yield
        ny_buf[...] = _dot(jnp.concatenate(_cmul(v[:NB], v[NB:], ny_tw[0], -ny_tw[1]), axis=1),
                           jnp.concatenate([_bf16(feat[12]), _bf16(feat[13])], axis=0))
        yield

    pieces = nyquist_column()
    spectra = {}
    for i in range(NA // 2 + 1):
        for c in range(2 * i, min(2 * i + 2, NA)):
            spectra[c] = _dot(_bf16(seq[0, c]), t_buf[c])
        if i in NYQUIST_AT:
            next(pieces)
        for c in range(max(2 * i - 2, 0), 2 * i):
            z = spectra.pop(c)
            words = [w_cls[part, c // 8, pl.ds(c % 8, NB, stride=8), :] for part in range(2)]
            w = [jnp.concatenate([pltpu.bitcast(v << 16, F32), pltpu.bitcast(v & -65536, F32)], axis=1)
                 for v in words]
            t_buf[c] = _dot(_bf16(seq[1, c]), jnp.concatenate(_cmul(z[:NB], z[NB:], *w), axis=0))
    fence()

    order = [k + 4 * i for k in range(4) for i in range(4)]
    pieces = out_projection(EARLY_OUT, S // 128)
    for r in range(NB // 8):
        nyquist = ny_buf[_span(r, 8), :]
        halves = []
        for parity in range(2):
            next(pieces)
            tiles = []
            for tile in range(2):
                z = _fft(lambda m: [t_buf[class_rows(m, parity, part, r, tile)] for part in range(2)],
                         list(range(HA)), 1)
                z = [_rotate(z[a], a * parity, NA, 1) for a in range(HA)]
                tiles.append([jnp.concatenate([z[a][part] for a in order], axis=0) for part in range(2)])
            (even_re, even_im), (odd_re, odd_im) = tiles
            slots = [HA * parity + a for a in order]
            last = jnp.concatenate([pltpu.roll(nyquist, 128 - s, 1) if s else nyquist for s in slots], axis=0)
            even_im = pltpu.roll(jnp.where(lanes == 0, last, even_im), 1, 1)
            ee = _dot(jnp.where(even_lane, even_re, even_im), _bf16(feat[5]))
            eo = _dot(jnp.where(even_lane, even_im, even_re), _bf16(feat[6]))
            odd_im = odd_im * lane_sign
            shared = _dot(odd_re + odd_im, _bf16(feat[7]))
            d0 = _dot(odd_re, _bf16(feat[8])) + shared
            d1 = _dot(odd_im, _bf16(feat[9])) + shared
            s0, s1 = eo + ee, ee - eo
            halves.append(jnp.concatenate([s0 + d0, s1 + d1, s0 - d0, s1 - d1], axis=1))
        for first, y in ((0, halves[0] + halves[1]), (HA, halves[0] - halves[1])):
            for i, a in enumerate(order):
                out_b[r, first + a] = _group(y, i).astype(BF16)
        out_b_copy(r).start()
    for _ in pieces:
        pass

    for cp in [out_a_copy(i) for i in range(S // 128)] + [out_b_copy(r) for r in range(NB // 8)]:
        cp.wait()


@jax.jit
def pallas_concat_heads__mha_block__spectral_gfnet__prompt_kernel(
    A_x: jax.Array,
    A_wqkv: jax.Array,
    A_wo: jax.Array,
    B_x: jax.Array,
    B_w_r: jax.Array,
    B_w_i: jax.Array,
):
    vmem = pltpu.VMEM
    out = pl.pallas_call(
        _kernel,
        out_shape=jax.ShapeDtypeStruct((NA, NB, 2 * D), BF16),
        in_specs=[pl.BlockSpec(memory_space=pltpu.HBM)] * 9,
        out_specs=pl.BlockSpec(memory_space=pltpu.HBM),
        scratch_shapes=[
            vmem((S, D), BF16), vmem((3, D, D), BF16), vmem((D, D), BF16), vmem((S, D), BF16),
            vmem((D // 2 + 1, S), BF16), vmem((D // 2 + 1, S), BF16),
            vmem(_FEAT.shape, I32), vmem(_SEQ.shape, I32), vmem(_NY_TW.shape, F32),
            vmem((3, D // 2, D), I32),
            vmem((D, S), F32),
            vmem((D // 2, S), I32),
            vmem((H, 96, S), jnp.int8),
            vmem((H, S, 128), jnp.int8),
            vmem((H, 8, S), F32),
            vmem((S // TK, H, 128), F32),
            vmem((D, S), F32),
            vmem((2, NA // 8, 8 * NB, 128), I32),
            vmem((NA, 2 * NB, 256), F32),
            vmem((NB, 128), F32),
            vmem((NA, NB, D), BF16),
            vmem((NB // 8, NA, 8, D), BF16),
            pltpu.SMEM((2,), I32),
            pltpu.SemaphoreType.DMA((5,)),
        ],
        compiler_params=pltpu.CompilerParams(vmem_limit_bytes=100 * 2 ** 20),
        name="mha_gfnet",
    )(A_x.reshape(S, D), A_wqkv, A_wo, B_x.reshape(S, D), B_w_r.T, B_w_i.T, _FEAT, _SEQ, _NY_TW)
    return out.reshape(1, S, 2 * D)
```

```python
import math

import jax
import jax.numpy as jnp
import numpy as np
from jax import lax
from jax.experimental import pallas as pl
from jax.experimental.pallas import tpu as pltpu

F32, BF16, I32 = jnp.float32, jnp.bfloat16, jnp.int32

S, D, H, DH = 2048, 512, 32, 16
TQ = 512
TK = 256
HEADS_PER_ITER = 4
NA, NB = 32, 64
HA = NA // 2

LOGIT_SCALE = DH ** -0.5 * math.log2(math.e)
QMAX = 3940.0
TINY = 1e-30
MAX_UNIT = 2.0 ** -12
MIN_DENOM, MAX_DENOM, MAX_FINITE = 2.0 ** -20, 2.0 ** 100, 3e38

TOKENS_IN = (256, 896, 896, S)
PROJECTION_PLAN = ("kk", "dkkkk", "kqqvqdvqvqqq",
                   "dvv" + "kdvvkqq" + "kdvvkqffq" * 2 + "kdvvkqffqffq" + "kdvvv")
EARLY_OUT = 6


def _dft_constants():
    def row_pairs(m):
        bits = m.astype(np.float32).astype(BF16).view(np.uint16).astype(np.uint32)
        return (bits[..., 0::2, :] | (bits[..., 1::2, :] << 16)).view(np.int32)

    n, m, l = np.arange(128)[:, None], np.arange(64)[None, :], np.arange(128)[None, :]
    angle = lambda k: 2 * np.pi * ((n * k) % D) / D
    ee, eo = np.zeros((128, 128)), np.zeros((128, 128))
    ee[:, 0::2], ee[:, 1::2] = np.cos(angle(4 * m)), -np.sin(angle(4 * m))
    ee[:, 1] = (-1.0) ** n[:, 0]
    eo[:, 1::2] = np.cos(angle(4 * m + 2))
    eo[:, 0::2] = np.roll(-np.sin(angle(4 * m + 2)), 1, axis=1)
    ga, gb = np.cos(angle(2 * l + 1)), -np.sin(angle(2 * l + 1)) * (-1.0) ** l
    twice = 2.0 / (S * D)
    ee_weight = np.where(n < 2, twice / 2, twice)
    forward = [ee, eo, ga, gb - ga, -(ga + gb)]
    inverse = [ee.T * ee_weight, eo.T * twice, gb.T * twice, (ga - gb).T * twice, -(ga + gb).T * twice]

    freq = np.arange(NA)[:, None, None] + NA * np.arange(NB)[None, :, None]
    th = 2 * np.pi * ((freq * np.arange(NB)[None, None, :]) % S) / S
    re, im = np.cos(th), -np.sin(th)
    seq = np.concatenate([np.concatenate([re, -im], axis=2), np.concatenate([im, re], axis=2)], axis=1)

    live = (n < NA) & (n // HA == l % 2)
    th = 2 * np.pi * (((n % HA) * l) % NA) / NA
    ny_re, ny_im = np.cos(th) * live, -np.sin(th) * live
    th = 2 * np.pi * (np.arange(NB)[:, None] * (l % NA)) / S
    return (row_pairs(np.stack(forward + inverse + [ny_re, ny_im, ny_re.T, ny_im.T])),
            row_pairs(np.stack([seq, seq.transpose(0, 2, 1)])),
            np.stack([np.cos(th), -np.sin(th)]).astype(np.float32))


_FEAT, _SEQ, _NY_TW = _dft_constants()


def _rotate(z, k, n, sign):
    re, im = z
    if k == 0:
        return z
    if 4 * k == n:
        return (-im, re) if sign > 0 else (im, -re)
    c, s = math.cos(2 * math.pi * k / n), sign * math.sin(2 * math.pi * k / n)
    if (8 * k) % n == 0 and (4 * k) % n != 0:
        return ((re - im) * c, (re + im) * c) if c * s > 0 else ((re + im) * c, (im - re) * c)
    return re * c - im * s, re * s + im * c


def _fft(load, idx, sign):
    n = len(idx)
    if n == 1:
        return [load(idx[0])]
    if n == 2:
        (ar, ai), (br, bi) = load(idx[0]), load(idx[1])
        return [(ar + br, ai + bi), (ar - br, ai - bi)]
    even, odd1, odd3 = (_fft(load, part, sign) for part in (idx[0::2], idx[1::4], idx[3::4]))
    out = [None] * n
    for k in range(n // 4):
        ar, ai = _rotate(odd1[k], k, n, sign)
        br, bi = _rotate(odd3[k], 3 * k, n, sign)
        sr, si, dr, di = ar + br, ai + bi, ar - br, ai - bi
        (er, ei), (fr, fi) = even[k], even[k + n // 4]
        out[k], out[k + n // 2] = (er + sr, ei + si), (er - sr, ei - si)
        plus, minus = (fr - di, fi + dr), (fr + di, fi - dr)
        out[k + n // 4], out[k + 3 * n // 4] = (plus, minus) if sign > 0 else (minus, plus)
    return out


def _fft_load_order(idx):
    if len(idx) <= 2:
        return idx
    return _fft_load_order(idx[0::2]) + _fft_load_order(idx[1::4]) + _fft_load_order(idx[3::4])


def _cmul(ar, ai, br, bi):
    return ar * br - ai * bi, ar * bi + ai * br


def _dot(a, b, contract=((1,), (0,)), out=F32):
    return lax.dot_general(a, b, (contract, ((), ())), preferred_element_type=out)


def _span(i, size):
    return pl.ds(i * size if isinstance(i, int) else pl.multiple_of(i * size, size), size)


def _group(v, i):
    return v[8 * i:8 * i + 8]


def _bf16(words):
    return pltpu.bitcast(words, BF16)


def _abs_max(t):
    return jnp.maximum(jnp.abs(t[:8]), jnp.abs(t[8:]))


def _digits(x):
    q = jnp.round(x).astype(I32)
    u = q + 128
    hi = u >> 8
    return hi << 3, hi, q, ((u & 255) - 120) >> 4


def _flip_groups(p):
    return jnp.concatenate([_group(p, 16 * a + g) for a in range(p.shape[0] // 128)
                            for g in range(15, -1, -1)], axis=0)


def _kernel(xa_hbm, wqkv_hbm, wo_hbm, xb_hbm, wr_hbm, wi_hbm, feat_hbm, seq_hbm, tw_hbm, out_hbm,
            xa, wqkv, wo, xb, wr, wi, feat, seq, ny_tw,
            w_t, k_t, v_t, q_dig, k_dig, q_max, k_unit, o_t,
            w_cls, t_buf, ny_buf, out_a, out_b, fence_buf, sem):
    def copy(src, dst, slot):
        return pltpu.make_async_copy(src, dst, sem.at[slot])

    def x_rows(lo, hi):
        return xa_hbm.at[pl.ds(lo, hi - lo)], xa.at[pl.ds(lo, hi - lo)]

    def w_part(part):
        return wqkv_hbm.at[:, _span(part, D)], wqkv.at[part]

    arrivals = [[copy(src, dst, slot) for src, dst in pairs] for slot, pairs in enumerate((
        [x_rows(0, TOKENS_IN[0]), w_part(1)],
        [x_rows(TOKENS_IN[0], TOKENS_IN[1])],
        [w_part(0), w_part(2)],
        [x_rows(TOKENS_IN[2], S), (wr_hbm, wr), (wi_hbm, wi)],
        [(xb_hbm, xb), (wo_hbm, wo), (feat_hbm, feat), (seq_hbm, seq), (tw_hbm, ny_tw)]))]
    for batch in arrivals:
        for cp in batch:
            cp.start()

    def arrive(slot):
        for cp in arrivals[slot]:
            cp.wait()

    def fence():
        def body(i, carry):
            fence_buf[i] = i
            return carry

        lax.fori_loop(0, 2, body, 0)

    def transpose_weights(part):
        for blk in range(D // 128):
            w_t[part, _span(blk, 64), :] = pltpu.bitcast(wqkv[part, :, _span(blk, 128)].T, I32)

    def project(part, x):
        return _dot(_bf16(w_t[part]), x, ((1,), (1,)))

    def queries(n):
        cols = _span(n, 128)
        y = project(0, xa[cols, :])
        for h in range(H):
            q = y[DH * h:DH * (h + 1)]
            m = jnp.maximum(jnp.max(_abs_max(q), axis=0, keepdims=True), TINY)
            q_max[h, :, cols] = jnp.broadcast_to(m, (8, 128))
            top, hi, lo, mid = _digits(q * (pltpu.reciprocal(m, approx=True) * QMAX))
            q_dig[h, :, cols] = jnp.concatenate(
                [top, top, lo, hi, mid, jnp.zeros_like(mid)], axis=0).astype(jnp.int8)

    def keys(n):
        k_t[:, _span(n, 128)] = project(1, jnp.concatenate(
            [xa[_span(16 * n + g, 8), :].astype(F32) for g in range(15, -1, -1)], axis=0))

    def values(n):
        v_t[:, _span(n, 128)] = pltpu.bitcast(project(2, xa[_span(n, 128), :]).astype(BF16), I32)

    def key_digits(t):
        cols = _span(t, TK)
        scales = []
        for g in range(H // 8):
            m = []
            for h in range(8 * g, 8 * g + 8):
                a = _abs_max(k_t[_span(h, DH), cols])
                m.append(jnp.max(jnp.maximum(a[:, :128], a[:, 128:]), axis=0, keepdims=True))
            m = jnp.max(jnp.concatenate(m, axis=0), axis=1, keepdims=True)
            m = jnp.maximum(jnp.broadcast_to(m, (8, 128)), TINY)
            k_unit[t, _span(g, 8), :] = m * (256.0 * LOGIT_SCALE / QMAX ** 2)
            scales.append(pltpu.reciprocal(m, approx=True) * QMAX)
        for h in range(H):
            scale = jnp.tile(scales[h // 8][h % 8:h % 8 + 1], (1, TK // 128))
            top, hi, lo, mid = _digits(k_t[_span(h, DH), cols] * scale)
            k_dig[h, cols, :] = jnp.concatenate(
                [top, top, top, top, hi, lo, mid, jnp.zeros_like(mid)],
                axis=0).astype(jnp.int16).T.astype(jnp.int8)

    def regroup_filter(i):
        for part, w in enumerate((wr, wi)):
            words = pltpu.bitcast(w[0:D // 2, _span(i, 256)], I32).T
            for e in range(256 // NA):
                for c8 in range(NA // 8):
                    w_cls[part, c8, _span(i * (256 // NA) + e, 8), :] = _group(words, NA // 8 * e + c8)

    tasks = dict(q=queries, k=keys, v=values, d=key_digits, f=regroup_filter)
    done = dict(q=0, k=0, v=0, d=0, f=0)
    for slot, new_weights in enumerate(((1,), (), (0, 2), ())):
        arrive(slot)
        for part in new_weights:
            transpose_weights(part)
        if slot == 3:
            fence()
        for name in PROJECTION_PLAN[slot]:
            assert name != "d" or 128 * done["k"] >= TK * (done["d"] + 1)
            assert name in "df" or 128 * (done[name] + 1) <= TOKENS_IN[slot]
            tasks[name](done[name])
            done[name] += 1
    assert done == dict(q=S // 128, k=S // 128, v=S // 128, d=S // TK, f=S // 256)
    arrive(4)

    def logits(h, j, t):
        top = q_dig[h, 0:32, _span(j, TQ)]
        digits = jnp.concatenate([top, top, q_dig[h, 32:96, _span(j, TQ)]], axis=0)
        return _dot(k_dig[h, _span(t, TK), :], digits, out=I32)

    def attend(it, failed):
        steps = [(it * HEADS_PER_ITER + i, j, t) for i in range(HEADS_PER_ITER)
                 for j in range(S // TQ) for t in range(S // TK)]
        y_next = logits(*steps[0])
        for n, (h, j, t) in enumerate(steps):
            y = y_next
            if n + 1 < len(steps):
                y_next = logits(*steps[n + 1])
            unit_k = jnp.broadcast_to(k_unit[t, pl.ds(h, 1), :], (8, 128))
            unit = q_max[h, :, _span(j, TQ)] * jnp.tile(unit_k, (1, TQ // 128))
            p = jnp.exp2(y.astype(F32).reshape(TK // 8, 8, TQ) * unit)
            den = jnp.sum(p, axis=0) if t == 0 else den + jnp.sum(p, axis=0)
            pv = _dot(_bf16(v_t[_span(h, DH // 2), _span(t, TK)]), _flip_groups(p.reshape(TK, TQ)))
            acc = pv if t == 0 else pv + acc
            coarsest = unit_k if t == 0 else jnp.maximum(coarsest, unit_k)
            if t == S // TK - 1:
                den = jnp.sum(den, axis=0, keepdims=True)
                o_t[_span(h, DH), _span(j, TQ)] = acc * (1.0 / den)
                ok = ((den >= MIN_DENOM) & (den <= MAX_DENOM) & (_abs_max(acc) <= MAX_FINITE)
                      & (q_max[h, :, _span(j, TQ)] * jnp.tile(coarsest, (1, TQ // 128)) <= MAX_UNIT))
                bad = jnp.where(ok, 0.0, 1.0)
                failed = failed + ((bad[:, 0:128] + bad[:, 128:256]) + (bad[:, 256:384] + bad[:, 384:512]))
        return failed

    failed = lax.fori_loop(0, H // HEADS_PER_ITER, attend, jnp.zeros((8, 128), F32))

    @pl.when(jnp.max(failed) > 0.0)
    def _():
        def attend_with_row_max(i, carry):
            h, cols = i // (S // TQ), _span(i % (S // TQ), TQ)
            q = _dot(_bf16(w_t[0, _span(h, DH // 2), :]), xa[cols, :], ((1,), (1,))).astype(BF16)

            def step(t, state):
                m_old, den, acc = state
                s = _dot(k_t[_span(h, DH), _span(t, TK)].astype(BF16), q, ((0,), (0,)))
                m = jnp.maximum(m_old, jnp.max(s, axis=0, keepdims=True))
                p = jnp.exp2((s - m) * LOGIT_SCALE)
                keep = jnp.exp2((m_old - m) * LOGIT_SCALE)
                pv = _dot(_bf16(v_t[_span(h, DH // 2), _span(t, TK)]), _flip_groups(p))
                return m, den * keep + jnp.sum(p, axis=0, keepdims=True), acc * keep + pv

            _, den, acc = lax.fori_loop(0, S // TK, step, (
                jnp.full((1, TQ), -jnp.inf, F32), jnp.zeros((1, TQ), F32), jnp.zeros((DH, TQ), F32)))
            o_t[_span(h, DH), cols] = acc / den
            return carry

        lax.fori_loop(0, H * (S // TQ), attend_with_row_max, 0)

    def out_a_copy(i):
        return copy(out_a.at[_span(i, 2)], out_hbm.at[_span(i, 2), :, pl.ds(0, D)], 0)

    def out_b_copy(r):
        return copy(out_b.at[r], out_hbm.at[:, _span(r, 8), pl.ds(D, D)], 0)

    def out_projection(first, last):
        for i in range(first, last):
            o = o_t[:, _span(i, 128)].astype(BF16).T
            for half in range(2):
                y = _dot(o, wo[:, _span(half, D // 2)]).astype(BF16)
                out_a[_span(i, 2), :, _span(half, D // 2)] = y.reshape(2, NB, D // 2)
                if half:
                    out_a_copy(i).start()
                yield

    lane = lax.broadcasted_iota(I32, (8, 128), 1)
    lanes = lax.broadcasted_iota(I32, (8 * HA, 128), 1)
    even_lane = (lanes & 1) == 0
    lane_sign = jnp.where(even_lane, 1.0, -1.0)

    def class_rows(m, parity, part, r, tile):
        return 2 * m + parity, _span(NB // 8 * part + r, 8), _span(tile, 128)

    order = _fft_load_order(list(range(HA)))
    pieces = out_projection(0, EARLY_OUT)
    for r in range(NB // 8):
        def tokens(first):
            return jnp.concatenate(
                [xb[_span(NB // 8 * (first + a) + r, 8), :].astype(F32) for a in order], axis=0)

        nyquist = jnp.zeros((8, 128), F32)
        for parity in range(2):
            x = tokens(0) - tokens(HA) if parity else tokens(0) + tokens(HA)
            x0, x1, x2, x3 = (x[:, 128 * i:128 * (i + 1)] for i in range(4))
            s0, s1, za, zb = x0 + x2, x1 + x3, x0 - x2, x3 - x1
            shared = _dot(za + zb, _bf16(feat[2]))
            odd_im = (_dot(za, _bf16(feat[3])) + shared) * lane_sign
            odd_re = _dot(zb, _bf16(feat[4])) + shared
            ee = _dot(s0 + s1, _bf16(feat[0]))
            eo = _dot(s0 - s1, _bf16(feat[1]))
            even_im = pltpu.roll(jnp.where(even_lane, eo, ee), 127, 1)
            for i, a in enumerate(order):
                slot, rows = HA * parity + a, _group(even_im, i)
                nyquist = jnp.where(lane == slot, pltpu.roll(rows, slot, 1) if slot else rows, nyquist)
            even = (jnp.where(even_lane, ee, eo), jnp.where(lanes == 0, 0.0, even_im))
            for tile, z in enumerate((even, (odd_re, odd_im))):
                spectrum = _fft(lambda a: _rotate([_group(v, order.index(a)) for v in z], a * parity, NA, -1),
                                list(range(HA)), -1)
                for m in range(HA):
                    for part in range(2):
                        t_buf[class_rows(m, parity, part, r, tile)] = spectrum[m][part]
        ny_buf[_span(r, 8), :] = nyquist
        for _ in range(2 - r % 2):
            next(pieces)
    assert next(pieces, "done") == "done"
    fence()

    def nyquist_filter(w):
        row = lax.broadcasted_iota(I32, (8, 128), 0)
        out = []
        for i in range(NB // 8):
            v = jnp.broadcast_to(w[D // 2:D // 2 + 1, _span(i, 256)].astype(F32), (8, 256))
            out.append(jnp.where((lane >> 5) == (row & 3), jnp.where(row < 4, v[:, :128], v[:, 128:]), 0.0))
        return jnp.concatenate(out, axis=0)

    def nyquist_column():
        v = _dot(ny_buf[...], jnp.concatenate([_bf16(feat[10]), _bf16(feat[11])], axis=1))
        yield
        v = _dot(_bf16(seq[0, 0]), jnp.concatenate(_cmul(v[:, :128], v[:, 128:], ny_tw[0], ny_tw[1]), axis=0))
        yield
        v = _dot(_bf16(seq[1, 0]), jnp.concatenate(
            _cmul(v[:NB], v[NB:], nyquist_filter(wr), nyquist_filter(wi)), axis=0))
        yield
        ny_buf[...] = _dot(jnp.concatenate(_cmul(v[:NB], v[NB:], ny_tw[0], -ny_tw[1]), axis=1),
                           jnp.concatenate([_bf16(feat[12]), _bf16(feat[13])], axis=0))
        yield

    pieces = nyquist_column()
    spectra = {}
    for i in range(NA // 2 + 1):
        for c in range(2 * i, min(2 * i + 2, NA)):
            spectra[c] = _dot(_bf16(seq[0, c]), t_buf[c])
        if i in (0, 2, 14, 16):
            next(pieces)
        for c in range(max(2 * i - 2, 0), 2 * i):
            z = spectra.pop(c)
            words = [w_cls[part, c // 8, pl.ds(c % 8, NB, stride=8), :] for part in range(2)]
            w = [jnp.concatenate([pltpu.bitcast(v << 16, F32), pltpu.bitcast(v & -65536, F32)], axis=1)
                 for v in words]
            t_buf[c] = _dot(_bf16(seq[1, c]), jnp.concatenate(_cmul(z[:NB], z[NB:], *w), axis=0))
    fence()

    order = [k + 4 * i for k in (0, 2, 1, 3) for i in (0, 2, 1, 3)]
    pieces = out_projection(EARLY_OUT, S // 128)
    for r in range(NB // 8):
        nyquist = ny_buf[_span(r, 8), :]
        halves = []
        for parity in range(2):
            next(pieces)
            tiles = []
            for tile in range(2):
                z = _fft(lambda m: [t_buf[class_rows(m, parity, part, r, tile)] for part in range(2)],
                         list(range(HA)), 1)
                z = [_rotate(z[a], a * parity, NA, 1) for a in range(HA)]
                tiles.append([jnp.concatenate([z[a][part] for a in order], axis=0) for part in range(2)])
            (even_re, even_im), (odd_re, odd_im) = tiles
            slots = [HA * parity + a for a in order]
            last = jnp.concatenate([pltpu.roll(nyquist, 128 - s, 1) if s else nyquist for s in slots], axis=0)
            even_im = pltpu.roll(jnp.where(lanes == 0, last, even_im), 1, 1)
            ee = _dot(jnp.where(even_lane, even_re, even_im), _bf16(feat[5]))
            eo = _dot(jnp.where(even_lane, even_im, even_re), _bf16(feat[6]))
            odd_im = odd_im * lane_sign
            shared = _dot(odd_re + odd_im, _bf16(feat[7]))
            d0 = _dot(odd_re, _bf16(feat[8])) + shared
            d1 = _dot(odd_im, _bf16(feat[9])) + shared
            s0, s1 = eo + ee, ee - eo
            halves.append(jnp.concatenate([s0 + d0, s1 + d1, s0 - d0, s1 - d1], axis=1))
        for first, y in ((0, halves[0] + halves[1]), (HA, halves[0] - halves[1])):
            for i, a in enumerate(order):
                out_b[r, first + a] = _group(y, i).astype(BF16)
        out_b_copy(r).start()
    for _ in pieces:
        pass

    for cp in [out_a_copy(i) for i in range(S // 128)] + [out_b_copy(r) for r in range(NB // 8)]:
        cp.wait()


@jax.jit
def pallas_concat_heads__mha_block__spectral_gfnet__prompt_kernel(
    A_x: jax.Array,
    A_wqkv: jax.Array,
    A_wo: jax.Array,
    B_x: jax.Array,
    B_w_r: jax.Array,
    B_w_i: jax.Array,
):
    vmem = pltpu.VMEM
    out = pl.pallas_call(
        _kernel,
        out_shape=jax.ShapeDtypeStruct((NA, NB, 2 * D), BF16),
        in_specs=[pl.BlockSpec(memory_space=pltpu.HBM)] * 9,
        out_specs=pl.BlockSpec(memory_space=pltpu.HBM),
        scratch_shapes=[
            vmem((S, D), BF16), vmem((3, D, D), BF16), vmem((D, D), BF16), vmem((S, D), BF16),
            vmem((D // 2 + 1, S), BF16), vmem((D // 2 + 1, S), BF16),
            vmem(_FEAT.shape, I32), vmem(_SEQ.shape, I32), vmem(_NY_TW.shape, F32),
            vmem((3, D // 2, D), I32),
            vmem((D, S), F32),
            vmem((D // 2, S), I32),
            vmem((H, 96, S), jnp.int8),
            vmem((H, S, 128), jnp.int8),
            vmem((H, 8, S), F32),
            vmem((S // TK, H, 128), F32),
            vmem((D, S), F32),
            vmem((2, NA // 8, 8 * NB, 128), I32),
            vmem((NA, 2 * NB, 256), F32),
            vmem((NB, 128), F32),
            vmem((NA, NB, D), BF16),
            vmem((NB // 8, NA, 8, D), BF16),
            pltpu.SMEM((2,), I32),
            pltpu.SemaphoreType.DMA((5,)),
        ],
        compiler_params=pltpu.CompilerParams(vmem_limit_bytes=100 * 2 ** 20),
        name="mha_gfnet",
    )(A_x.reshape(S, D), A_wqkv, A_wo, B_x.reshape(S, D), B_w_r.T, B_w_i.T, _FEAT, _SEQ, _NY_TW)
    return out.reshape(1, S, 2 * D)
```
